```python
import jax
import jax.numpy as jnp

def _softmax(x, axis=-1):
    return jax.nn.softmax(x, axis=axis)

def _gelu(x):
    return jax.nn.gelu(x, approximate=True)

def _silu(x):
    return jax.nn.silu(x)

def _sigmoid(x):
    return jax.nn.sigmoid(x)

def _layernorm(x, axis=-1, eps=1e-05):
    m = jnp.mean(x, axis=axis, keepdims=True)
    v = jnp.var(x, axis=axis, keepdims=True)
    return (x - m) / jnp.sqrt(v + eps)

def _scatter_add(tgt, idx, src, axis=0):
    return tgt.at[idx].add(src)

def _segment_sum(src, seg, n):
    return jax.ops.segment_sum(src, seg, n)

class _Rng:

    def __init__(self, key):
        self._k = key

    def _next(self):
        self._k, sub = jax.random.split(self._k)
        return sub

    def normal(self, shape):
        return jax.random.normal(self._next(), shape, dtype=jnp.bfloat16)

    def randint(self, lo, hi, shape):
        return jax.random.randint(self._next(), shape, lo, hi, dtype=jnp.int32)

    def uniform(self, shape, lo=0.0, hi=1.0):
        return jax.random.uniform(self._next(), shape, jnp.bfloat16, lo, hi)

    def permutation(self, n):
        return jax.random.permutation(self._next(), n)
kernel_name = 'adaLN_cond__mha_block_cached__moe_arch_mod__prompt'

def setup_inputs():
    _rng = _Rng(jax.random.key(int.from_bytes(__import__("os").urandom(4), "little")))
    _w = lambda a: (lambda t: t.astype(jnp.bfloat16) if jnp.issubdtype(t.dtype, jnp.floating) else t)(jnp.asarray(a))

    def _A_setup():
        B, Sq, D = (1, 2048, 1024)
        H, Sk, Dh = (32, 2048, 128)
        return {'x': _w((lambda *s: _rng.normal(s) * 0.05)(B, Sq, D)), 'k_cache': _w((lambda *s: _rng.normal(s) * 0.05)(B, H, Sk, Dh)), 'v_cache': _w((lambda *s: _rng.normal(s) * 0.05)(B, H, Sk, Dh)), 'wq': _w((lambda *s: _rng.normal(s) * 0.05)(D, H * Dh) * D ** (-0.5)), 'wo': _w((lambda *s: _rng.normal(s) * 0.05)(H * Dh, D) * (H * Dh) ** (-0.5))}
    _A_in = _A_setup()

    def _B_setup():
        B, S, D, F, C = (1, 2048, 1024, 3584, 2)
        return {'x': _w((lambda *s: _rng.normal(s) * 0.05)(B, S, D)), 'w_r': _w((lambda *s: _rng.normal(s) * 0.05)(D)), 'w_gate': _w((lambda *s: _rng.normal(s) * 0.05)(D, F)), 'w_up': _w((lambda *s: _rng.normal(s) * 0.05)(D, F)), 'w_down': _w((lambda *s: _rng.normal(s) * 0.05)(F, D))}
    _B_in = _B_setup()
    return {'A_x': _A_in['x'], 'A_k_cache': _A_in['k_cache'], 'A_v_cache': _A_in['v_cache'], 'A_wq': _A_in['wq'], 'A_wo': _A_in['wo'], 'B_x': _B_in['x'], 'B_w_r': _B_in['w_r'], 'B_w_gate': _B_in['w_gate'], 'B_w_up': _B_in['w_up'], 'B_w_down': _B_in['w_down'], 'c': _w((lambda *s: _rng.normal(s) * 0.05)(1, 1024)), 'w_mod': _w((lambda *s: _rng.normal(s) * 0.05)(1024, 6 * 1024) * 1024 ** (-0.5))}

def reference(A_x, A_k_cache, A_v_cache, A_wq, A_wo, B_x, B_w_r, B_w_gate, B_w_up, B_w_down, c, w_mod):

    def _A_ref(x, k_cache, v_cache, wq, wo):
        B, Sq, D = x.shape
        H, Dh = (32, 128)
        q = (lambda x, *d: x.transpose(*d))((x @ wq).reshape(B, Sq, H, Dh), 0, 2, 1, 3)
        scores = jnp.einsum('bhqd,bhkd->bhqk', q, k_cache) * Dh ** (-0.5)
        p = _softmax(scores, axis=-1)
        o = jnp.einsum('bhqk,bhkd->bhqd', p, v_cache)
        return (lambda x, *d: x.transpose(*d))(o, 0, 2, 1, 3).reshape(B, Sq, H * Dh) @ wo

    def _B_ref(x, w_r, w_gate, w_up, w_down):
        B, S, D = x.shape
        C = 2
        r = x @ w_r
        idx = jnp.argsort(-r, axis=-1)[:, :C]
        idx_e = jnp.repeat(idx.reshape(B, C, 1), D, axis=2)
        x_sel = jnp.take_along_axis(x, idx_e, axis=1)
        g = _silu(x_sel @ w_gate)
        u = x_sel @ w_up
        y = g * u @ w_down
        r_sel = _sigmoid(jnp.take_along_axis(r, idx, axis=1))
        y = y * r_sel.reshape(B, C, 1)
        b_off = (jnp.arange(B) * S).reshape(B, 1)
        flat_idx = (idx + b_off).reshape(B * C)
        zero = (x * 0.0).reshape(B * S, D)
        upd = _scatter_add(zero, flat_idx, y.reshape(B * C, D), axis=0)
        return x + upd.reshape(B, S, D)
    x = A_x
    mod = (_silu(c) @ w_mod).reshape(c.shape[0], 6, 1, -1)
    sa, ca, ga, sb, cb, gb = (mod[:, 0].copy(), mod[:, 1].copy(), mod[:, 2].copy(), mod[:, 3].copy(), mod[:, 4].copy(), mod[:, 5].copy())
    h = _layernorm(x, axis=-1) * (1 + ca) + sa
    x = x + ga * _A_ref(h, A_k_cache, A_v_cache, A_wq, A_wo)
    h = _layernorm(x, axis=-1) * (1 + cb) + sb
    x = x + gb * _B_ref(h, B_w_r, B_w_gate, B_w_up, B_w_down)
    return x
```

```python
import functools, contextlib
import jax
import jax.numpy as jnp
from jax import lax
import jax.experimental.pallas as pl
import jax.experimental.pallas.tpu as pltpu

S, D, H, DH, F = 2048, 1024, 32, 128, 3584
BF, F32, I32 = jnp.bfloat16, jnp.float32, jnp.int32
LOG2E = 1.4426950408889634
QSCALE = (DH ** -0.5) * LOG2E
KT = D // 128


def ldb(ref, *idx):
    return pltpu.bitcast(ref.bitcast(I32)[idx], BF)


def nt(a, b):
    return lax.dot_general(a, b, (((1,), (1,)), ((), ())), preferred_element_type=F32)


def nn(a, b):
    return jnp.dot(a, b, preferred_element_type=F32)


def rb(x):
    return x.astype(BF).astype(F32)


def rows(start, size):
    if isinstance(start, int):
        return pl.ds(start // 2, size // 2)
    return pl.ds(pl.multiple_of(start // 2, size // 2), size // 2)


def layernorm(x):
    m = jnp.mean(x, axis=-1, keepdims=True)
    xc = x - m
    v = jnp.mean(xc * xc, axis=-1, keepdims=True)
    return xc * lax.rsqrt(v + 1e-5)


def tile(x, j):
    return x[:, j * 128:(j + 1) * 128]


def make_kernel(cq=128, gk=256, la=1, opos=50, ec=256, mm=0, fuse_o=0, scopes=0, nloop=None, wo_t=1, static=0,
                qla=1, qpos=0, xc=256, do_epi=1, HP=1, cpy=1, nomod=0, order='', chunks='', ola=1):
    if chunks:
        CH = []
        for part in str(chunks).split('+'):
            n, sz = part.split('x')
            CH += [int(sz)] * int(n)
        assert sum(CH) == S
    else:
        CH = [cq] * (S // cq)
    OFF = [sum(CH[:i]) for i in range(len(CH))]
    NC = len(CH)
    NG = S // gk
    NP = H // HP
    nloop = NP if nloop is None else nloop
    MT = 4 * KT // NP

    def kernel(c_hbm, wr_hbm, x_hbm, k_hbm, v_hbm, wq_hbm, wo_hbm, wg_hbm, wu_hbm, wd_hbm, wmod_hbm,
               out_hbm,
               c_s, wr_s, x_s, h_s, o_s, acc_s, k_s, v_s, wq_s, wo_s, wot_s, wg_s, wu_s, wd_s, wma_s, wmb_s, mod_s,
               kw_s, vw_s, wqw_s,
               sem_h, sem_m, sem_x, sem_o, sem_w):
        scope = (lambda n: jax.named_scope(n)) if scopes else (lambda n: contextlib.nullcontext())
        copy = pltpu.make_async_copy
        cp_c = copy(c_hbm, c_s, sem_m.at[0])
        cp_wr = copy(wr_hbm, wr_s, sem_m.at[1])
        cp_sa = copy(wmod_hbm.at[:, pl.ds(0, D)], wma_s.at[:, pl.ds(0, D)], sem_m.at[2])
        cp_ca = copy(wmod_hbm.at[:, pl.ds(D, D)], wma_s.at[:, pl.ds(D, D)], sem_m.at[3])
        cp_g = copy(wg_hbm, wg_s, sem_m.at[4])
        cp_u = copy(wu_hbm, wu_s, sem_m.at[5])
        cp_d = copy(wd_hbm, wd_s, sem_m.at[6])
        NX = S // xc

        def cp_x(c):
            return copy(x_hbm.at[pl.ds(c * xc, xc)], x_s.at[pl.ds(c * xc, xc)], sem_x.at[c])

        def pair_copies(i, p):
            def col(h):
                return pl.ds(pl.multiple_of(h * DH, DH), DH)
            h = HP * i
            mcol = pl.ds(pl.multiple_of(2 * D + i * MT * 128, 128), MT * 128)
            q = 0 if cpy else p
            return ([copy(wq_hbm.at[:, col(h + k)], wq_s.at[q, k], sem_h.at[q, 3 + k]) for k in range(HP)] +
                    [copy(k_hbm.at[pl.ds(h, HP)], k_s.at[q], sem_h.at[q, 0]),
                     copy(v_hbm.at[pl.ds(h, HP)], v_s.at[q], sem_h.at[q, 1]),
                     copy(wo_hbm.at[pl.ds(pl.multiple_of(h * DH, HP * DH), HP * DH), :], wo_s.at[q], sem_h.at[q, 2]),
                     copy(wmod_hbm.at[:, mcol], wmb_s.at[p], sem_w.at[p])])

        for cp in [cp_c, cp_sa, cp_ca] + [cp_x(c) for c in range(NX)] + pair_copies(0, 0) + [cp_wr]:
            cp.start()

        acc_s[...] = jnp.zeros_like(acc_s)

        with scope("sc_p0_c"):
            cp_c.wait()
        c = c_s[...].astype(F32)
        sc = jnp.broadcast_to((c * jax.nn.sigmoid(c)).astype(BF), (16, D))

        def mod_vec(k):
            return jnp.concatenate([mod_s[k * KT + j, 0:1, :] for j in range(KT)], axis=1)

        for k, cp in enumerate((cp_sa, cp_ca)):
          with scope(f"sc_p1_mod{k}"):
            cp.wait()
            mk = rb(nn(sc, wma_s[:, k * D:(k + 1) * D])[0:8])
            for j in range(KT):
                mod_s[k * KT + j] = tile(mk, j)

        for i in range(NX):
          with scope(f"sc_p2_ln{i}"):
            cp_x(i).wait()

            def ln1(r, _, i=i):
                rs = pl.ds(pl.multiple_of(i * xc + r * 64, 64), 64)
                hh = layernorm(x_s[rs, :].astype(F32)) * (1.0 + mod_vec(1)) + mod_vec(0)
                for j in range(KT):
                    h_s[j, rs, :] = tile(hh, j).astype(BF)
                return _
            if xc == 64:
                ln1(0, 0)
            else:
                rs = pl.ds(i * xc, xc)
                hh = layernorm(x_s[rs, :].astype(F32)) * (1.0 + mod_vec(1)) + mod_vec(0)
                for j in range(KT):
                    h_s[j, rs, :] = tile(hh, j).astype(BF)

        def cp_out(i, n):
            r = i * n if isinstance(i, int) else pl.multiple_of(i * n, n)
            return copy(o_s.at[pl.ds(r, n)], out_hbm.at[pl.ds(r, n)], sem_o.at[i])

        def epilogue(i, n, attn, top):
            r0 = i * n if isinstance(i, int) else pl.multiple_of(i * n, n)
            rs = pl.ds(r0, n)
            x1b = (x_s[rs, :].astype(F32) + mod_vec(2) * attn).astype(BF)
            x_s[rs, :] = x1b
            x1 = x1b.astype(F32)
            m = jnp.mean(x1, axis=-1, keepdims=True)
            xcen = x1 - m
            rstd = lax.rsqrt(jnp.mean(xcen * xcen, axis=-1, keepdims=True) + 1e-5)
            cb1, sb, gb = 1.0 + mod_vec(4), mod_vec(3), mod_vec(5)
            xn = xcen * rstd
            o_s[rs, :] = ((x1 + gb * sb) + xn * (gb * cb1)).astype(BF)
            cp_out(i, n).start()
            wr = wr_s[...].astype(F32)
            r = rb(jnp.sum(xn * (cb1 * wr), axis=-1, keepdims=True) + jnp.sum(sb * wr, axis=-1, keepdims=True))
            sub = lax.broadcasted_iota(I32, (8, 128), 0)
            b1, i1, b2, i2 = top
            for t in range(n // 8):
                rv = jnp.broadcast_to(r[t * 8:(t + 1) * 8], (8, 128))
                iv = sub + (r0 + t * 8)
                g1 = rv > b1
                g2 = rv > b2
                b2 = jnp.where(g1, b1, jnp.where(g2, rv, b2))
                i2 = jnp.where(g1, i1, jnp.where(g2, iv, i2))
                b1 = jnp.where(g1, rv, b1)
                i1 = jnp.where(g1, iv, i1)
            return b1, i1, b2, i2

        def top_init():
            sub = lax.broadcasted_iota(I32, (8, 128), 0)
            ninf = jnp.full((8, 128), -jnp.inf, F32)
            return ninf, sub, ninf, sub + 8

        def prefetch(i, p):
            @pl.when(i + 1 < nloop)
            def _():
                for cp in pair_copies(i + 1, 1 - p):
                    cp.start()
            pl.when(i == 0)(cp_g.start)
            pl.when(i == 1)(cp_u.start)
            pl.when(i == 2)(cp_d.start)

        def pair_body(i, p):
            T = HP * NC
            q = 0 if cpy else p
            qs, ss, ms, ls, accs, os_ = {}, {}, {}, {}, {}, {}

            def qproj(t):
                k, c = divmod(t, NC)
                hh = jnp.concatenate([ldb(h_s, j, rows(OFF[c], CH[c]), slice(None)) for j in range(KT)], axis=1)
                if cpy and t >= qla:
                    w = ldb(wqw_s, k, slice(None), slice(None))
                else:
                    w = ldb(wq_s, q, k, slice(None), slice(None))
                qs[t] = (nn(hh, w) * QSCALE).astype(BF)

            def qk(t, g):
                kk = ldb(kw_s, t // NC, rows(g * gk, gk), slice(None)) if cpy else ldb(k_s, p, t // NC, rows(g * gk, gk), slice(None))
                s = nt(qs[t], kk)
                if not mm:
                    m = tile(s, 0)
                    for u in range(1, gk // 128):
                        m = jnp.maximum(m, tile(s, u))
                    ms[t] = m if g == 0 else jnp.maximum(ms[t], m)
                    if g == NG - 1:
                        ms[t] = jnp.max(ms[t], axis=-1, keepdims=True)
                ss[t, g] = s

            def pv(t, g):
                if mm and g == 0:
                    m = None
                    for gg in range(NG):
                        for u in range(gk // 128):
                            m = tile(ss[t, gg], u) if m is None else jnp.maximum(m, tile(ss[t, gg], u))
                    ms[t] = jnp.max(m, axis=-1, keepdims=True)
                pr = jnp.exp2(ss.pop((t, g)) - ms[t])
                l = tile(pr, 0)
                for u in range(1, gk // 128):
                    l = l + tile(pr, u)
                ls[t] = l if g == 0 else ls[t] + l
                vv = ldb(vw_s, t // NC, rows(g * gk, gk), slice(None)) if cpy else ldb(v_s, p, t // NC, rows(g * gk, gk), slice(None))
                o = nn(pr.astype(BF), vv)
                accs[t] = o if g == 0 else accs[t] + o
                if g == NG - 1:
                    l = jnp.sum(ls.pop(t), axis=-1, keepdims=True)
                    os_[t] = (accs.pop(t) * pl.reciprocal(l, approx=True)).astype(BF)

            def wo_tiles(k):
                if wo_t:
                    return jnp.concatenate([ldb(wot_s, j, rows(k * DH, DH), slice(None)) for j in range(KT)], axis=1)
                return wo_s[p, k * DH:(k + 1) * DH, :]

            def oproj(t):
                k, c = divmod(t, NC)
                rs = pl.ds(OFF[c], CH[c])
                if t == 0 and wo_t and not cpy:
                    for j in range(KT):
                        wot_s[j] = wo_s[p, :, j * 128:(j + 1) * 128]
                if fuse_o:
                    if k == 1:
                        o2 = jnp.concatenate([os_.pop(c), os_.pop(t)], axis=1)
                        wo = jnp.concatenate([wo_tiles(0), wo_tiles(1)], axis=0)
                        acc_s[rs, :] += nn(o2, wo)
                else:
                    acc_s[rs, :] += nn(os_.pop(t), wo_tiles(k))

            def mod_tiles():
                mk = rb(nn(sc, wmb_s[p])[0:8])
                for j in range(MT):
                    mod_s[2 * KT + i * MT + j] = tile(mk, j)

            og = max(NG * opos // 100 - 1, 0)
            qg = NG * qpos // 100
            for t in range(qla):
                qproj(t)
            if cpy:
                for k in range(HP):
                    wqw_s[k] = ldb(wq_s, 0, k, slice(None), slice(None))
                for k in range(HP):
                    kw_s[k] = ldb(k_s, 0, k, slice(None), slice(None))
                for k in range(HP):
                    vw_s[k] = ldb(v_s, 0, k, slice(None), slice(None))
                for j in range(KT):
                    wot_s[j] = wo_s[0, :, j * 128:(j + 1) * 128]
                prefetch(i, p)
            for t in range(T + la + ola):
              with (scope(f"sc_{t:02d}") if scopes > 1 else contextlib.nullcontext()):
                if order:
                    for ch in order:
                        if ch == 'Q' and t + qla < T:
                            qproj(t + qla)
                        if ch == 'K' and t < T:
                            qk(t, 0)
                        if ch == 'V' and 0 <= t - la < T:
                            pv(t - la, 0)
                        if ch == 'O' and 0 <= t - la - ola < T:
                            oproj(t - la - ola)
                for g in range(NG if not order else 0):
                    if g == qg and t + qla < T:
                        qproj(t + qla)
                    if t < T:
                        qk(t, g)
                    if 0 <= t - la < T:
                        pv(t - la, g)
                    if g == og and 0 <= t - la - 1 < T:
                        oproj(t - la - 1)
                if t == NC // 2 and not nomod:
                    mod_tiles()

        def loop(i, _):
            p = i % 2

            if not cpy:
                prefetch(i, p)
            for cp in pair_copies(i, p):
                cp.wait()
            pair_body(i, p)
            return _

        with scope("sc_p3_loop"):
            lax.fori_loop(0, nloop, loop, None)
        cp_wr.wait()

        def epi(i, top):
            return epilogue(i, ec, acc_s[pl.ds(pl.multiple_of(i * ec, ec), ec), :], top)
        with scope("sc_p4_epi"):
            top = lax.fori_loop(0, S // ec, epi, top_init())

        with scope("sc_tail0"):
            b1, i1, b2, i2 = top
            m0 = jnp.max(b1, axis=0, keepdims=True)
            j0 = jnp.min(jnp.where(b1 == m0, i1, S - 1), axis=0, keepdims=True)
            won = i1 == j0
            cb, ci = jnp.where(won, b2, b1), jnp.where(won, i2, i1)
            m1 = jnp.max(cb, axis=0, keepdims=True)
            j1 = jnp.min(jnp.where(cb == m1, ci, S - 1), axis=0, keepdims=True)
            r0, r1 = jnp.max(j0), jnp.max(j1)
            b0_ = pl.multiple_of((r0 // 16) * 16, 16)
            b1_ = pl.multiple_of((r1 // 16) * 16, 16)
            sub = lax.broadcasted_iota(I32, (16, D), 0)

            def pick(base, i):
                slab = x_s[pl.ds(base, 16), :].astype(F32)
                return jnp.sum(jnp.where(sub == i - base, slab, 0.0), axis=0, keepdims=True)

            x1 = jnp.where(sub == 0, pick(b0_, r0), jnp.where(sub == 1, pick(b1_, r1), 0.0))
            h2 = layernorm(x1) * (1.0 + mod_vec(4)) + mod_vec(3)
            xs = h2.astype(BF)
        with scope("sc_tail1"):
            cp_g.wait()
            cp_u.wait()
            cp_d.wait()
            g = rb(nn(xs, wg_s[...]))
            u = rb(nn(xs, wu_s[...]))
            a = (rb(g * jax.nn.sigmoid(g)) * u).astype(BF)
            y = rb(nn(a, wd_s[...]))
            y = y * jax.nn.sigmoid(jnp.where(sub == 0, m0[:, 0:1], m1[:, 0:1]))
            new = x1 + mod_vec(5) * (h2 + y)
        with scope("sc_tail2"):
            for i in range(S // ec):
                cp_out(i, ec).wait()
            for k, (base, i) in enumerate(((b0_, r0), (b1_, r1))):
                row = jnp.sum(jnp.where(sub == k, new, 0.0), axis=0, keepdims=True)
                o_s[pl.ds(base, 16), :] = jnp.where(sub == i - base, row.astype(BF), o_s[pl.ds(base, 16), :])
            p0 = copy(o_s.at[pl.ds(b0_, 16)], out_hbm.at[pl.ds(b0_, 16)], sem_o.at[0])
            p1 = copy(o_s.at[pl.ds(b1_, 16)], out_hbm.at[pl.ds(b1_, 16)], sem_o.at[1])
            p0.start()

            @pl.when(b1_ != b0_)
            def _():
                p1.start()
                p1.wait()
            p0.wait()

    scratch = [
        pltpu.VMEM((1, D), BF),
        pltpu.VMEM((1, D), BF),
        pltpu.VMEM((S, D), BF),
        pltpu.VMEM((KT, S, 128), BF),
        pltpu.VMEM((S, D), BF),
        pltpu.VMEM((S, D), F32),
        pltpu.VMEM((2, HP, S, DH), BF),
        pltpu.VMEM((2, HP, S, DH), BF),
        pltpu.VMEM((2, HP, D, DH), BF),
        pltpu.VMEM((2, HP * DH, D), BF),
        pltpu.VMEM((KT, HP * DH, 128), BF),
        pltpu.VMEM((D, F), BF),
        pltpu.VMEM((D, F), BF),
        pltpu.VMEM((F, D), BF),
        pltpu.VMEM((D, 2 * D), BF),
        pltpu.VMEM((2, D, MT * 128), BF),
        pltpu.VMEM((6 * KT, 8, 128), F32),
        pltpu.VMEM((HP, S, DH), BF),
        pltpu.VMEM((HP, S, DH), BF),
        pltpu.VMEM((HP, D, DH), BF),
        pltpu.SemaphoreType.DMA((2, 3 + HP)),
        pltpu.SemaphoreType.DMA((7,)),
        pltpu.SemaphoreType.DMA((32,)),
        pltpu.SemaphoreType.DMA((32,)),
        pltpu.SemaphoreType.DMA((2,)),
    ]
    return kernel, scratch


def build(**cfg):
    fl = cfg.pop('fl', '')
    nb = cfg.pop('nb', 0)
    names = dict(lp="XLA_TPU_FORCE_LP_LLO_SCHEDULER", even="XLA_TPU_EVENLY_DISTRIBUTE_CRITICAL_NODES",
                 dma="XLA_TPU_RESCHEDULE_DMA_DONES", flat="XLA_TPU_ENABLE_LLO_SMALL_LOOP_FLATTENING")
    flags = {names[x]: True for x in str(fl).split('+') if x} or None
    kernel, scratch = make_kernel(**cfg)

    @jax.jit
    def fn(A_x, A_k_cache, A_v_cache, A_wq, A_wo, B_x, B_w_r, B_w_gate, B_w_up, B_w_down, c, w_mod):
        hbm = pl.BlockSpec(memory_space=pl.ANY)
        out = pl.pallas_call(
            kernel,
            out_shape=jax.ShapeDtypeStruct((S, D), BF),
            in_specs=[hbm] * 11,
            out_specs=hbm,
            scratch_shapes=scratch,
            compiler_params=pltpu.CompilerParams(vmem_limit_bytes=120 * 1024 * 1024, flags=flags,
                                                 disable_bounds_checks=bool(nb)),
        )(c, B_w_r.reshape(1, D), A_x.reshape(S, D), A_k_cache.reshape(H, S, DH), A_v_cache.reshape(H, S, DH),
          A_wq, A_wo, B_w_gate, B_w_up, B_w_down, w_mod)
        return out.reshape(1, S, D)
    return fn


_impl = build(**{'nb': 1, 'gk': 2048, 'mm': 1, 'order': 'QKVO', 'chunks': '32x64', 'ola': 2})


@jax.jit
def pallas_adaLN_cond__mha_block_cached__moe_arch_mod__prompt_kernel(
    A_x, A_k_cache, A_v_cache, A_wq, A_wo, B_x, B_w_r, B_w_gate, B_w_up, B_w_down, c, w_mod
):
    return _impl(A_x, A_k_cache, A_v_cache, A_wq, A_wo, B_x, B_w_r, B_w_gate, B_w_up, B_w_down, c, w_mod)
```

```python
import functools, contextlib
import jax
import jax.numpy as jnp
from jax import lax
import jax.experimental.pallas as pl
import jax.experimental.pallas.tpu as pltpu

S, D, H, DH, F = 2048, 1024, 32, 128, 3584
BF, F32, I32 = jnp.bfloat16, jnp.float32, jnp.int32
LOG2E = 1.4426950408889634
QSCALE = (DH ** -0.5) * LOG2E
KT = D // 128


def ldb(ref, *idx):
    return pltpu.bitcast(ref.bitcast(I32)[idx], BF)


def nt(a, b):
    return lax.dot_general(a, b, (((1,), (1,)), ((), ())), preferred_element_type=F32)


def nn(a, b):
    return jnp.dot(a, b, preferred_element_type=F32)


def rb(x):
    return x.astype(BF).astype(F32)


def rows(start, size):
    if isinstance(start, int):
        return pl.ds(start // 2, size // 2)
    return pl.ds(pl.multiple_of(start // 2, size // 2), size // 2)


def layernorm(x):
    m = jnp.mean(x, axis=-1, keepdims=True)
    xc = x - m
    v = jnp.mean(xc * xc, axis=-1, keepdims=True)
    return xc * lax.rsqrt(v + 1e-5)


def tile(x, j):
    return x[:, j * 128:(j + 1) * 128]


def make_kernel(cq=128, gk=256, la=1, opos=50, ec=256, mm=0, fuse_o=0, scopes=0, nloop=None, wo_t=1, static=0,
                qla=1, qpos=0, xc=256, do_epi=1, HP=1, cpy=1, nomod=0, mxmean=0, order='', chunks='', ola=1):
    if chunks:
        CH = []
        for part in str(chunks).split('+'):
            n, sz = part.split('x')
            CH += [int(sz)] * int(n)
        assert sum(CH) == S
    else:
        CH = [cq] * (S // cq)
    OFF = [sum(CH[:i]) for i in range(len(CH))]
    NC = len(CH)
    NG = S // gk
    NP = H // HP
    nloop = NP if nloop is None else nloop
    MT = 4 * KT // NP

    def kernel(c_hbm, wr_hbm, x_hbm, k_hbm, v_hbm, wq_hbm, wo_hbm, wg_hbm, wu_hbm, wd_hbm, wmod_hbm,
               out_hbm,
               c_s, wr_s, x_s, h_s, o_s, acc_s, k_s, v_s, wq_s, wo_s, wot_s, wg_s, wu_s, wd_s, wma_s, wmb_s, mod_s,
               kw_s, vw_s, wqw_s, vec_s, w1_s,
               sem_h, sem_m, sem_x, sem_o, sem_w):
        scope = (lambda n: jax.named_scope(n)) if scopes else (lambda n: contextlib.nullcontext())
        copy = pltpu.make_async_copy
        cp_c = copy(c_hbm, c_s, sem_m.at[0])
        cp_wr = copy(wr_hbm, wr_s, sem_m.at[1])
        cp_sa = copy(wmod_hbm.at[:, pl.ds(0, D)], wma_s.at[:, pl.ds(0, D)], sem_m.at[2])
        cp_ca = copy(wmod_hbm.at[:, pl.ds(D, D)], wma_s.at[:, pl.ds(D, D)], sem_m.at[3])
        cp_g = copy(wg_hbm, wg_s, sem_m.at[4])
        cp_u = copy(wu_hbm, wu_s, sem_m.at[5])
        cp_d = copy(wd_hbm, wd_s, sem_m.at[6])
        NX = S // xc

        def cp_x(c):
            r = c * xc if isinstance(c, int) else pl.multiple_of(c * xc, xc)
            return copy(x_hbm.at[pl.ds(r, xc)], x_s.at[pl.ds(r, xc)], sem_x.at[c])

        def pair_copies(i, p):
            def col(h):
                return pl.ds(pl.multiple_of(h * DH, DH), DH)
            h = HP * i
            mcol = pl.ds(pl.multiple_of(2 * D + i * MT * 128, 128), MT * 128)
            q = 0 if cpy else p
            return ([copy(wq_hbm.at[:, col(h + k)], wq_s.at[q, k], sem_h.at[q, 3 + k]) for k in range(HP)] +
                    [copy(k_hbm.at[pl.ds(h, HP)], k_s.at[q], sem_h.at[q, 0]),
                     copy(v_hbm.at[pl.ds(h, HP)], v_s.at[q], sem_h.at[q, 1]),
                     copy(wo_hbm.at[pl.ds(pl.multiple_of(h * DH, HP * DH), HP * DH), :], wo_s.at[q], sem_h.at[q, 2]),
                     copy(wmod_hbm.at[:, mcol], wmb_s.at[p], sem_w.at[p])])

        for cp in [cp_c, cp_sa, cp_ca] + [cp_x(c) for c in range(NX)] + pair_copies(0, 0) + [cp_wr]:
            cp.start()

        acc_s[...] = jnp.zeros_like(acc_s)

        with scope("sc_p0_c"):
            cp_c.wait()
        c = c_s[...].astype(F32)
        sc = jnp.broadcast_to((c * jax.nn.sigmoid(c)).astype(BF), (16, D))

        def wr_vec():
            w = wr_s[...].astype(F32)
            return jnp.concatenate([w[j:j + 1, :] for j in range(KT)], axis=1)

        def mod_vec(k):
            return jnp.concatenate([mod_s[k * KT + j, 0:1, :] for j in range(KT)], axis=1)

        for k, cp in enumerate((cp_sa, cp_ca)):
          with scope(f"sc_p1_mod{k}"):
            cp.wait()
            mk = rb(nn(sc, wma_s[:, k * D:(k + 1) * D])[0:8])
            for j in range(KT):
                mod_s[k * KT + j] = tile(mk, j)

        def ln1(i, _):
            cp_x(i).wait()
            rs = pl.ds(pl.multiple_of(i * xc, xc), xc)
            hh = layernorm(x_s[rs, :].astype(F32)) * (1.0 + mod_vec(1)) + mod_vec(0)
            for j in range(KT):
                h_s[j, rs, :] = tile(hh, j).astype(BF)
            return _
        with scope("sc_p2_ln"):
            lax.fori_loop(0, NX, ln1, None)

        def cp_out(i, n):
            r = i * n if isinstance(i, int) else pl.multiple_of(i * n, n)
            return copy(o_s.at[pl.ds(r, n)], out_hbm.at[pl.ds(r, n)], sem_o.at[i])

        def rows_ds(i, n):
            return pl.ds(i * n, n) if isinstance(i, int) else pl.ds(pl.multiple_of(i * n, n), n)

        def stage_a(i, n):
            rs = rows_ds(i, n)
            x1 = x_s[rs, :].astype(F32) + vec_s[0] * acc_s[rs, :]
            acc_s[rs, :] = x1
            if mxmean:
                return nn(x1.astype(BF), jnp.full((D, 128), 1.0 / D, BF))[:, 0:1]
            return jnp.mean(x1, axis=-1, keepdims=True)

        def stage_b(i, n, m):
            d = acc_s[rows_ds(i, n), :] - m
            return lax.rsqrt(jnp.mean(d * d, axis=-1, keepdims=True) + 1e-5)

        def stage_c(i, n, m, rstd, top):
            rs = rows_ds(i, n)
            r0 = i * n
            x1 = acc_s[rs, :]
            xn = (x1 - m) * rstd
            o_s[rs, :] = (x1 + (xn * vec_s[1] + vec_s[2])).astype(BF)
            cp_out(i, n).start()
            r = rb(nt(w1_s[...], xn.astype(BF))[0:8] + vec_s[4, :, 0:1])
            lane = lax.broadcasted_iota(I32, (8, 128), 1)
            b1, i1, b2, i2 = top
            for t in range(n // 128):
                rv = tile(r, t)
                iv = lane + (r0 + t * 128)
                g1 = rv > b1
                g2 = rv > b2
                b2 = jnp.where(g1, b1, jnp.where(g2, rv, b2))
                i2 = jnp.where(g1, i1, jnp.where(g2, iv, i2))
                b1 = jnp.where(g1, rv, b1)
                i1 = jnp.where(g1, iv, i1)
            return b1, i1, b2, i2

        def top_init():
            lane = lax.broadcasted_iota(I32, (8, 128), 1)
            ninf = jnp.full((8, 128), -jnp.inf, F32)
            return ninf, lane, ninf, lane + 128

        def prefetch(i, p):
            @pl.when(i + 1 < nloop)
            def _():
                for cp in pair_copies(i + 1, 1 - p):
                    cp.start()
            pl.when(i == 0)(cp_g.start)
            pl.when(i == 1)(cp_u.start)
            pl.when(i == 2)(cp_d.start)

        def pair_body(i, p):
            T = HP * NC
            q = 0 if cpy else p
            qs, ss, ms, ls, accs, os_ = {}, {}, {}, {}, {}, {}

            def qproj(t):
                k, c = divmod(t, NC)
                hh = jnp.concatenate([ldb(h_s, j, rows(OFF[c], CH[c]), slice(None)) for j in range(KT)], axis=1)
                if cpy and t >= qla:
                    w = ldb(wqw_s, k, slice(None), slice(None))
                else:
                    w = ldb(wq_s, q, k, slice(None), slice(None))
                qs[t] = (nn(hh, w) * QSCALE).astype(BF)

            def qk(t, g):
                kk = ldb(kw_s, t // NC, rows(g * gk, gk), slice(None)) if cpy else ldb(k_s, p, t // NC, rows(g * gk, gk), slice(None))
                s = nt(qs[t], kk)
                if not mm:
                    m = tile(s, 0)
                    for u in range(1, gk // 128):
                        m = jnp.maximum(m, tile(s, u))
                    ms[t] = m if g == 0 else jnp.maximum(ms[t], m)
                    if g == NG - 1:
                        ms[t] = jnp.max(ms[t], axis=-1, keepdims=True)
                ss[t, g] = s

            def pv(t, g):
                if mm and g == 0:
                    m = None
                    for gg in range(NG):
                        for u in range(gk // 128):
                            m = tile(ss[t, gg], u) if m is None else jnp.maximum(m, tile(ss[t, gg], u))
                    ms[t] = jnp.max(m, axis=-1, keepdims=True)
                pr = jnp.exp2(ss.pop((t, g)) - ms[t])
                l = tile(pr, 0)
                for u in range(1, gk // 128):
                    l = l + tile(pr, u)
                ls[t] = l if g == 0 else ls[t] + l
                vv = ldb(vw_s, t // NC, rows(g * gk, gk), slice(None)) if cpy else ldb(v_s, p, t // NC, rows(g * gk, gk), slice(None))
                o = nn(pr.astype(BF), vv)
                accs[t] = o if g == 0 else accs[t] + o
                if g == NG - 1:
                    l = jnp.sum(ls.pop(t), axis=-1, keepdims=True)
                    os_[t] = (accs.pop(t) * pl.reciprocal(l, approx=True)).astype(BF)

            def wo_tiles(k):
                if wo_t:
                    return jnp.concatenate([ldb(wot_s, j, rows(k * DH, DH), slice(None)) for j in range(KT)], axis=1)
                return wo_s[p, k * DH:(k + 1) * DH, :]

            def oproj(t):
                k, c = divmod(t, NC)
                rs = pl.ds(OFF[c], CH[c])
                if t == 0 and wo_t and not cpy:
                    for j in range(KT):
                        wot_s[j] = wo_s[p, :, j * 128:(j + 1) * 128]
                if fuse_o:
                    if k == 1:
                        o2 = jnp.concatenate([os_.pop(c), os_.pop(t)], axis=1)
                        wo = jnp.concatenate([wo_tiles(0), wo_tiles(1)], axis=0)
                        acc_s[rs, :] += nn(o2, wo)
                else:
                    acc_s[rs, :] += nn(os_.pop(t), wo_tiles(k))

            def mod_tiles():
                mk = rb(nn(sc, wmb_s[p])[0:8])
                for j in range(MT):
                    mod_s[2 * KT + i * MT + j] = tile(mk, j)

            og = max(NG * opos // 100 - 1, 0)
            qg = NG * qpos // 100
            for t in range(qla):
                qproj(t)
            if cpy:
                wqw_s.bitcast(I32)[...] = wq_s.bitcast(I32)[0]
                kw_s.bitcast(I32)[...] = k_s.bitcast(I32)[0]
                vw_s.bitcast(I32)[...] = v_s.bitcast(I32)[0]
                for j in range(KT):
                    wot_s[j] = wo_s[0, :, j * 128:(j + 1) * 128]
                prefetch(i, p)
            for t in range(T + la + ola):
              with (scope(f"sc_{t:02d}") if scopes > 1 else contextlib.nullcontext()):
                if order:
                    for ch in order:
                        if ch == 'Q' and t + qla < T:
                            qproj(t + qla)
                        if ch == 'K' and t < T:
                            qk(t, 0)
                        if ch == 'V' and 0 <= t - la < T:
                            pv(t - la, 0)
                        if ch == 'O' and 0 <= t - la - ola < T:
                            oproj(t - la - ola)
                for g in range(NG if not order else 0):
                    if g == qg and t + qla < T:
                        qproj(t + qla)
                    if t < T:
                        qk(t, g)
                    if 0 <= t - la < T:
                        pv(t - la, g)
                    if g == og and 0 <= t - la - 1 < T:
                        oproj(t - la - 1)
                if t == NC // 2 and not nomod:
                    mod_tiles()

        def loop(i, _):
            p = i % 2

            if not cpy:
                prefetch(i, p)
            if scopes:
                @pl.when(i > 0)
                def _():
                    for cp in pair_copies(i, p):
                        cp.wait()
            else:
                for cp in pair_copies(i, p):
                    cp.wait()
            pair_body(i, p)
            return _

        if scopes:
            with scope("sc_p2b_wait"):
                for cp in pair_copies(0, 0):
                    cp.wait()
        with scope("sc_p3_loop"):
            lax.fori_loop(0, nloop, loop, None)
        cp_wr.wait()

        with scope("sc_p4_epi"):
            ga, sb, cb1, gb = mod_vec(2), mod_vec(3), 1.0 + mod_vec(4), mod_vec(5)
            wr = wr_vec()
            vec_s[0] = ga
            vec_s[1] = gb * cb1
            vec_s[2] = gb * sb
            w1_s[...] = jnp.broadcast_to(cb1 * wr, (16, D)).astype(BF)
            vec_s[4] = jnp.broadcast_to(jnp.sum(sb * wr, axis=-1, keepdims=True), (1, D))
            NE = S // ec
            m0_ = stage_a(0, ec)
            m1_ = stage_a(1, ec)
            r0_ = stage_b(0, ec, m0_)

            def epi(i, carry):
                ma, mb, rb_, top = carry
                mc = stage_a(i, ec)
                rc = stage_b(i - 1, ec, mb)
                top = stage_c(i - 2, ec, ma, rb_, top)
                return mb, mc, rc, top

            def bc(v):
                return jnp.broadcast_to(v, (ec, 128))[:, 0:1] if False else v
            ma, mb, rb_, top = lax.fori_loop(2, NE, epi, (m0_, m1_, r0_, top_init()))
            rc = stage_b(NE - 1, ec, mb)
            top = stage_c(NE - 2, ec, ma, rb_, top)
            top = stage_c(NE - 1, ec, mb, rc, top)

        with scope("sc_tail0"):
            b1, i1, b2, i2 = top
            m0 = jnp.max(b1, axis=1, keepdims=True)
            j0 = jnp.min(jnp.where(b1 == m0, i1, S - 1), axis=1, keepdims=True)
            won = i1 == j0
            cb, ci = jnp.where(won, b2, b1), jnp.where(won, i2, i1)
            m1 = jnp.max(cb, axis=1, keepdims=True)
            j1 = jnp.min(jnp.where(cb == m1, ci, S - 1), axis=1, keepdims=True)
            r0, r1 = jnp.max(j0), jnp.max(j1)
            b0_ = pl.multiple_of((r0 // 16) * 16, 16)
            b1_ = pl.multiple_of((r1 // 16) * 16, 16)
            sub = lax.broadcasted_iota(I32, (16, D), 0)

            def pick(base, i):
                slab = acc_s[pl.ds(base, 16), :]
                return jnp.sum(jnp.where(sub == i - base, slab, 0.0), axis=0, keepdims=True)

            x1 = jnp.where(sub == 0, pick(b0_, r0), jnp.where(sub == 1, pick(b1_, r1), 0.0))
            h2 = layernorm(x1) * (1.0 + mod_vec(4)) + mod_vec(3)
            xs = h2.astype(BF)
        with scope("sc_tail1"):
            cp_g.wait()
            cp_u.wait()
            cp_d.wait()
            g = rb(nn(xs, wg_s[...]))
            u = rb(nn(xs, wu_s[...]))
            a = (rb(g * jax.nn.sigmoid(g)) * u).astype(BF)
            y = rb(nn(a, wd_s[...]))
            y = y * jax.nn.sigmoid(jnp.where(sub == 0, m0[0:1, 0:1], m1[0:1, 0:1]))
            new = x1 + mod_vec(5) * (h2 + y)
        with scope("sc_tail2"):
            for i in range(S // ec):
                cp_out(i, ec).wait()
            for k, (base, i) in enumerate(((b0_, r0), (b1_, r1))):
                row = jnp.sum(jnp.where(sub == k, new, 0.0), axis=0, keepdims=True)
                o_s[pl.ds(base, 16), :] = jnp.where(sub == i - base, row.astype(BF), o_s[pl.ds(base, 16), :])
            p0 = copy(o_s.at[pl.ds(b0_, 16)], out_hbm.at[pl.ds(b0_, 16)], sem_o.at[0])
            p1 = copy(o_s.at[pl.ds(b1_, 16)], out_hbm.at[pl.ds(b1_, 16)], sem_o.at[1])
            p0.start()

            @pl.when(b1_ != b0_)
            def _():
                p1.start()
                p1.wait()
            p0.wait()

    scratch = [
        pltpu.VMEM((1, D), BF),
        pltpu.VMEM((KT, 128), BF),
        pltpu.VMEM((S, D), BF),
        pltpu.VMEM((KT, S, 128), BF),
        pltpu.VMEM((S, D), BF),
        pltpu.VMEM((S, D), F32),
        pltpu.VMEM((1, HP, S, DH), BF),
        pltpu.VMEM((1, HP, S, DH), BF),
        pltpu.VMEM((1, HP, D, DH), BF),
        pltpu.VMEM((1, HP * DH, D), BF),
        pltpu.VMEM((KT, HP * DH, 128), BF),
        pltpu.VMEM((D, F), BF),
        pltpu.VMEM((D, F), BF),
        pltpu.VMEM((F, D), BF),
        pltpu.VMEM((D, 2 * D), BF),
        pltpu.VMEM((2, D, MT * 128), BF),
        pltpu.VMEM((6 * KT, 8, 128), F32),
        pltpu.VMEM((HP, S, DH), BF),
        pltpu.VMEM((HP, S, DH), BF),
        pltpu.VMEM((HP, D, DH), BF),
        pltpu.VMEM((5, 1, D), F32),
        pltpu.VMEM((16, D), BF),
        pltpu.SemaphoreType.DMA((2, 3 + HP)),
        pltpu.SemaphoreType.DMA((7,)),
        pltpu.SemaphoreType.DMA((32,)),
        pltpu.SemaphoreType.DMA((64,)),
        pltpu.SemaphoreType.DMA((2,)),
    ]
    return kernel, scratch


def build(**cfg):
    fl = cfg.pop('fl', '')
    nb = cfg.pop('nb', 0)
    names = dict(lp="XLA_TPU_FORCE_LP_LLO_SCHEDULER", even="XLA_TPU_EVENLY_DISTRIBUTE_CRITICAL_NODES",
                 dma="XLA_TPU_RESCHEDULE_DMA_DONES", flat="XLA_TPU_ENABLE_LLO_SMALL_LOOP_FLATTENING")
    flags = {names[x]: True for x in str(fl).split('+') if x} or None
    kernel, scratch = make_kernel(**cfg)

    @jax.jit
    def fn(A_x, A_k_cache, A_v_cache, A_wq, A_wo, B_x, B_w_r, B_w_gate, B_w_up, B_w_down, c, w_mod):
        hbm = pl.BlockSpec(memory_space=pl.ANY)
        out = pl.pallas_call(
            kernel,
            out_shape=jax.ShapeDtypeStruct((S, D), BF),
            in_specs=[hbm] * 11,
            out_specs=hbm,
            scratch_shapes=scratch,
            compiler_params=pltpu.CompilerParams(vmem_limit_bytes=120 * 1024 * 1024, flags=flags,
                                                 disable_bounds_checks=bool(nb)),
        )(c, B_w_r.reshape(KT, 128), A_x.reshape(S, D), A_k_cache.reshape(H, S, DH), A_v_cache.reshape(H, S, DH),
          A_wq, A_wo, B_w_gate, B_w_up, B_w_down, w_mod)
        return out.reshape(1, S, D)
    return fn


_impl = build(**{'nb': 1, 'gk': 2048, 'mm': 1, 'order': 'QKVO', 'chunks': '32x64', 'ola': 2, 'HP': 2, 'ec': 256, 'qla': 2})


@jax.jit
def pallas_adaLN_cond__mha_block_cached__moe_arch_mod__prompt_kernel(
    A_x, A_k_cache, A_v_cache, A_wq, A_wo, B_x, B_w_r, B_w_gate, B_w_up, B_w_down, c, w_mod
):
    return _impl(A_x, A_k_cache, A_v_cache, A_wq, A_wo, B_x, B_w_r, B_w_gate, B_w_up, B_w_down, c, w_mod)
```

```python
import jax
import jax.numpy as jnp
from jax import lax
import jax.experimental.pallas as pl
import jax.experimental.pallas.tpu as pltpu

S, D, H, DH, F = 2048, 1024, 32, 128, 3584
BF, F32, I32 = jnp.bfloat16, jnp.float32, jnp.int32
LOG2E = 1.4426950408889634
QSCALE = (DH ** -0.5) * LOG2E
EPS = 1e-5
KT = D // 128
HP = 2
NP = H // HP
CQ = 64
NC = S // CQ
QLAG, VLAG, OLAG = 2, 1, 3
MT = 4 * KT // NP
XC = 512
EC = 256
NX, NE = S // XC, S // EC


def _ldb(ref, *idx):
    return pltpu.bitcast(ref.bitcast(I32)[idx], BF)


def _nt(a, b):
    return lax.dot_general(a, b, (((1,), (1,)), ((), ())), preferred_element_type=F32)


def _nn(a, b):
    return jnp.dot(a, b, preferred_element_type=F32)


def _rb(x):
    return x.astype(BF).astype(F32)


def _tile(x, j):
    return x[:, j * 128:(j + 1) * 128]


def _blk(i, n):
    return pl.ds(i * n, n) if isinstance(i, int) else pl.ds(pl.multiple_of(i * n, n), n)


def _layernorm(x):
    m = jnp.mean(x, axis=-1, keepdims=True)
    xc = x - m
    v = jnp.mean(xc * xc, axis=-1, keepdims=True)
    return xc * lax.rsqrt(v + EPS)


def _kernel(c_hbm, wr_hbm, x_hbm, k_hbm, v_hbm, wq_hbm, wo_hbm, wg_hbm, wu_hbm, wd_hbm, wmod_hbm,
            out_hbm,
            c_s, wr_s, x_s, h_s, o_s, acc_s,
            k_st, v_st, wq_st, wo_st,
            k_s, v_s, wq_s, wo_s,
            wg_s, wu_s, wd_s, wma_s, wmb_s, mod_s, vec_s, w1_s,
            sem_h, sem_m, sem_x, sem_o, sem_w):
    copy = pltpu.make_async_copy
    cp_c = copy(c_hbm, c_s, sem_m.at[0])
    cp_wr = copy(wr_hbm, wr_s, sem_m.at[1])
    cp_sa = copy(wmod_hbm.at[:, pl.ds(0, D)], wma_s.at[:, pl.ds(0, D)], sem_m.at[2])
    cp_ca = copy(wmod_hbm.at[:, pl.ds(D, D)], wma_s.at[:, pl.ds(D, D)], sem_m.at[3])
    cp_g = copy(wg_hbm, wg_s, sem_m.at[4])
    cp_u = copy(wu_hbm, wu_s, sem_m.at[5])
    cp_d = copy(wd_hbm, wd_s, sem_m.at[6])

    def cp_x(i):
        return copy(x_hbm.at[_blk(i, XC)], x_s.at[_blk(i, XC)], sem_x.at[i])

    def cp_out(i):
        return copy(o_s.at[_blk(i, EC)], out_hbm.at[_blk(i, EC)], sem_o.at[i])

    def pair_copies(i):
        h = HP * i
        return ([copy(wq_hbm.at[:, _blk(h + k, DH)], wq_st.at[k], sem_h.at[3 + k]) for k in range(HP)] +
                [copy(k_hbm.at[pl.ds(h, HP)], k_st, sem_h.at[0]),
                 copy(v_hbm.at[pl.ds(h, HP)], v_st, sem_h.at[1]),
                 copy(wo_hbm.at[_blk(i, HP * DH), :], wo_st, sem_h.at[2])])

    def mod_copy(j, p):
        col = pl.ds(pl.multiple_of(2 * D + j * MT * 128, 128), MT * 128)
        return copy(wmod_hbm.at[:, col], wmb_s.at[p], sem_w.at[p])

    for cp in [cp_c, cp_sa, cp_ca] + [cp_x(i) for i in range(NX)] + pair_copies(0) + [cp_wr]:
        cp.start()

    acc_s[...] = jnp.zeros_like(acc_s)
    wmb_s[0] = jnp.zeros((D, MT * 128), BF)

    cp_c.wait()
    c = c_s[...].astype(F32)
    sc = jnp.broadcast_to((c * jax.nn.sigmoid(c)).astype(BF), (16, D))

    def mod_vec(k):
        return jnp.concatenate([mod_s[k * KT + j, 0:1, :] for j in range(KT)], axis=1)

    for k, cp in enumerate((cp_sa, cp_ca)):
        cp.wait()
        mk = _rb(_nn(sc, wma_s[:, k * D:(k + 1) * D])[0:8])
        for j in range(KT):
            mod_s[k * KT + j] = _tile(mk, j)

    def ln1(i, carry):
        cp_x(i).wait()
        rs = _blk(i, XC)
        hh = _layernorm(x_s[rs, :].astype(F32)) * (1.0 + mod_vec(1)) + mod_vec(0)
        for j in range(KT):
            h_s[j, rs, :] = _tile(hh, j).astype(BF)
        return carry

    lax.fori_loop(0, NX, ln1, None)

    def mod_slice(p, base):
        mk = _rb(_nn(sc, wmb_s[p])[0:8])
        for j in range(MT):
            mod_s[base + j] = _tile(mk, j)

    def pair(i, carry):
        p = i % 2
        for cp in pair_copies(i):
            cp.wait()
        pl.when(i > 0)(mod_copy(jnp.maximum(i - 1, 0), p).wait)

        T = HP * NC
        qs, ss, os_ = {}, {}, {}

        def rows(c_):
            return pl.ds(c_ * CQ // 2, CQ // 2)

        def qproj(t, wq_ref):
            k, c_ = divmod(t, NC)
            hh = jnp.concatenate([_ldb(h_s, j, rows(c_), slice(None)) for j in range(KT)], axis=1)
            qs[t] = (_nn(hh, _ldb(wq_ref, k, slice(None), slice(None))) * QSCALE).astype(BF)

        def qk(t):
            ss[t] = _nt(qs.pop(t), _ldb(k_s, t // NC, slice(0, S // 2), slice(None)))

        def pv(t):
            s = ss.pop(t)
            m = _tile(s, 0)
            for u in range(1, S // 128):
                m = jnp.maximum(m, _tile(s, u))
            m = jnp.max(m, axis=-1, keepdims=True)
            pr = jnp.exp2(s - m)
            l = _tile(pr, 0)
            for u in range(1, S // 128):
                l = l + _tile(pr, u)
            o = _nn(pr.astype(BF), _ldb(v_s, t // NC, slice(0, S // 2), slice(None)))
            l = jnp.sum(l, axis=-1, keepdims=True)
            os_[t] = (o * pl.reciprocal(l, approx=False)).astype(BF)

        def oproj(t):
            k, c_ = divmod(t, NC)
            w = jnp.concatenate(
                [_ldb(wo_s, j, pl.ds(k * DH // 2, DH // 2), slice(None)) for j in range(KT)], axis=1)
            acc_s[pl.ds(c_ * CQ, CQ), :] += _nn(os_.pop(t), w)

        for t in range(QLAG):
            qproj(t, wq_st)
        wq_s.bitcast(I32)[...] = wq_st.bitcast(I32)[...]
        k_s.bitcast(I32)[...] = k_st.bitcast(I32)[...]
        v_s.bitcast(I32)[...] = v_st.bitcast(I32)[...]
        for j in range(KT):
            wo_s[j] = wo_st[:, j * 128:(j + 1) * 128]

        @pl.when(i + 1 < NP)
        def _():
            for cp in pair_copies(i + 1):
                cp.start()
        mod_copy(i, 1 - p).start()
        pl.when(i == 0)(cp_g.start)
        pl.when(i == 1)(cp_u.start)
        pl.when(i == 2)(cp_d.start)

        for t in range(T + OLAG):
            if t + QLAG < T:
                qproj(t + QLAG, wq_s)
            if t < T:
                qk(t)
            if 0 <= t - VLAG < T:
                pv(t - VLAG)
            if 0 <= t - OLAG < T:
                oproj(t - OLAG)
            if t == 0:
                mod_slice(p, jnp.where(i == 0, 6 * KT, 2 * KT + (i - 1) * MT))
        return carry

    lax.fori_loop(0, NP, pair, None)
    cp_wr.wait()
    mod_copy(NP - 1, NP % 2).wait()
    mod_slice(NP % 2, 2 * KT + (NP - 1) * MT)

    def stage_a(i):
        rs = _blk(i, EC)
        x1 = x_s[rs, :].astype(F32) + vec_s[0] * acc_s[rs, :]
        acc_s[rs, :] = x1
        return jnp.mean(x1, axis=-1, keepdims=True)

    def stage_b(i, m):
        d = acc_s[_blk(i, EC), :] - m
        return lax.rsqrt(jnp.mean(d * d, axis=-1, keepdims=True) + EPS)

    lane = lax.broadcasted_iota(I32, (8, 128), 1)

    def stage_c(i, m, rstd, top):
        rs = _blk(i, EC)
        x1 = acc_s[rs, :]
        xn = (x1 - m) * rstd
        o_s[rs, :] = (x1 + (xn * vec_s[1] + vec_s[2])).astype(BF)
        cp_out(i).start()
        r = _rb(_nt(w1_s[...], xn.astype(BF))[0:8] + vec_s[3, :, 0:1])
        b1, i1, b2, i2 = top
        for t in range(EC // 128):
            rv = _tile(r, t)
            iv = lane + (i * EC + t * 128)
            g1 = rv > b1
            g2 = rv > b2
            b2 = jnp.where(g1, b1, jnp.where(g2, rv, b2))
            i2 = jnp.where(g1, i1, jnp.where(g2, iv, i2))
            b1 = jnp.where(g1, rv, b1)
            i1 = jnp.where(g1, iv, i1)
        return b1, i1, b2, i2

    wr = wr_s[...].astype(F32)
    wr = jnp.concatenate([wr[j:j + 1, :] for j in range(KT)], axis=1)
    ga, sb, cb1, gb = mod_vec(2), mod_vec(3), 1.0 + mod_vec(4), mod_vec(5)
    vec_s[0] = ga
    vec_s[1] = gb * cb1
    vec_s[2] = gb * sb
    vec_s[3] = jnp.broadcast_to(jnp.sum(sb * wr, axis=-1, keepdims=True), (1, D))
    w1_s[...] = jnp.broadcast_to(cb1 * wr, (16, D)).astype(BF)

    ninf = jnp.full((8, 128), -jnp.inf, F32)
    m_a = stage_a(0)
    m_b = stage_a(1)
    r_a = stage_b(0, m_a)

    def epi(i, carry):
        ma, mb, ra, top = carry
        mc = stage_a(i)
        rb = stage_b(i - 1, mb)
        top = stage_c(i - 2, ma, ra, top)
        return mb, mc, rb, top

    ma, mb, ra, top = lax.fori_loop(2, NE, epi, (m_a, m_b, r_a, (ninf, lane, ninf, lane + 128)))
    rb = stage_b(NE - 1, mb)
    top = stage_c(NE - 2, ma, ra, top)
    b1, i1, b2, i2 = stage_c(NE - 1, mb, rb, top)

    m0 = jnp.max(b1, axis=1, keepdims=True)
    j0 = jnp.min(jnp.where(b1 == m0, i1, S - 1), axis=1, keepdims=True)
    won = i1 == j0
    cb, ci = jnp.where(won, b2, b1), jnp.where(won, i2, i1)
    m1 = jnp.max(cb, axis=1, keepdims=True)
    j1 = jnp.min(jnp.where(cb == m1, ci, S - 1), axis=1, keepdims=True)
    r0, r1 = jnp.max(j0), jnp.max(j1)
    s0 = pl.multiple_of((r0 // 16) * 16, 16)
    s1 = pl.multiple_of((r1 // 16) * 16, 16)
    sub = lax.broadcasted_iota(I32, (16, D), 0)

    def pick(base, r):
        return jnp.sum(jnp.where(sub == r - base, acc_s[pl.ds(base, 16), :], 0.0), axis=0, keepdims=True)

    x1 = jnp.where(sub == 0, pick(s0, r0), jnp.where(sub == 1, pick(s1, r1), 0.0))
    h2 = _layernorm(x1) * cb1 + sb
    xs = h2.astype(BF)
    cp_g.wait()
    cp_u.wait()
    cp_d.wait()
    g = _rb(_nn(xs, wg_s[...]))
    u = _rb(_nn(xs, wu_s[...]))
    a = (_rb(g * jax.nn.sigmoid(g)) * u).astype(BF)
    y = _rb(_nn(a, wd_s[...]))
    y = y * jax.nn.sigmoid(jnp.where(sub == 0, m0[0:1, 0:1], m1[0:1, 0:1]))
    new = x1 + gb * (h2 + y)

    for i in range(NE):
        cp_out(i).wait()
    for k, (base, r) in enumerate(((s0, r0), (s1, r1))):
        row = jnp.sum(jnp.where(sub == k, new, 0.0), axis=0, keepdims=True)
        o_s[pl.ds(base, 16), :] = jnp.where(sub == r - base, row.astype(BF), o_s[pl.ds(base, 16), :])
    p0 = copy(o_s.at[pl.ds(s0, 16)], out_hbm.at[pl.ds(s0, 16)], sem_o.at[0])
    p1 = copy(o_s.at[pl.ds(s1, 16)], out_hbm.at[pl.ds(s1, 16)], sem_o.at[1])
    p0.start()

    @pl.when(s1 != s0)
    def _():
        p1.start()
        p1.wait()
    p0.wait()


@jax.jit
def pallas_adaLN_cond__mha_block_cached__moe_arch_mod__prompt_kernel(
    A_x, A_k_cache, A_v_cache, A_wq, A_wo, B_x, B_w_r, B_w_gate, B_w_up, B_w_down, c, w_mod
):
    del B_x
    vmem = pltpu.VMEM
    dma = pltpu.SemaphoreType.DMA
    scratch = [
        vmem((1, D), BF),
        vmem((KT, 128), BF),
        vmem((S, D), BF),
        vmem((KT, S, 128), BF),
        vmem((S, D), BF),
        vmem((S, D), F32),
        vmem((HP, S, DH), BF), vmem((HP, S, DH), BF), vmem((HP, D, DH), BF), vmem((HP * DH, D), BF),
        vmem((HP, S, DH), BF), vmem((HP, S, DH), BF), vmem((HP, D, DH), BF), vmem((KT, HP * DH, 128), BF),
        vmem((D, F), BF), vmem((D, F), BF), vmem((F, D), BF),
        vmem((D, 2 * D), BF),
        vmem((2, D, MT * 128), BF),
        vmem((6 * KT + MT, 8, 128), F32),
        vmem((4, 1, D), F32),
        vmem((16, D), BF),
        dma((3 + HP,)), dma((7,)), dma((NX,)), dma((NE,)), dma((2,)),
    ]
    out = pl.pallas_call(
        _kernel,
        out_shape=jax.ShapeDtypeStruct((S, D), BF),
        in_specs=[pl.BlockSpec(memory_space=pl.ANY)] * 11,
        out_specs=pl.BlockSpec(memory_space=pl.ANY),
        scratch_shapes=scratch,
        compiler_params=pltpu.CompilerParams(
            vmem_limit_bytes=120 * 1024 * 1024, disable_bounds_checks=True),
    )(c, B_w_r.reshape(KT, 128), A_x.reshape(S, D), A_k_cache.reshape(H, S, DH),
      A_v_cache.reshape(H, S, DH), A_wq, A_wo, B_w_gate, B_w_up, B_w_down, w_mod)
    return out.reshape(1, S, D)
```
